```python
import os as _os
_os.environ.setdefault("JAX_PLATFORMS", "cpu")
import jax
import jax.numpy as jnp

def _softmax(x, axis=-1):
    return jax.nn.softmax(x, axis=axis)
def _gelu(x):
    return jax.nn.gelu(x, approximate=True)
def _silu(x):
    return jax.nn.silu(x)
def _sigmoid(x):
    return jax.nn.sigmoid(x)
def _layernorm(x, axis=-1, eps=1e-5):
    m = jnp.mean(x, axis=axis, keepdims=True)
    v = jnp.var(x, axis=axis, keepdims=True)
    return (x - m) / jnp.sqrt(v + eps)
def _scatter_add(tgt, idx, src, axis=0):
    return tgt.at[idx].add(src)
def _segment_sum(src, seg, n):
    return jax.ops.segment_sum(src, seg, n)
class _Rng:
    def __init__(self, key):
        self._k = key
    def _next(self):
        self._k, sub = jax.random.split(self._k)
        return sub
    def normal(self, shape):
        return jax.random.normal(self._next(), shape, dtype=jnp.bfloat16)
    def randint(self, lo, hi, shape):
        return jax.random.randint(self._next(), shape, lo, hi, dtype=jnp.int32)
    def uniform(self, shape, lo=0.0, hi=1.0):
        return jax.random.uniform(self._next(), shape, jnp.bfloat16, lo, hi)
    def permutation(self, n):
        return jax.random.permutation(self._next(), n)


kernel_name = 'standalone__dcn_v2_cross__recsys'

def setup_inputs():
    _rng = _Rng(jax.random.key(int.from_bytes(__import__("os").urandom(4), "little")))
    _w = (lambda a: (lambda t: t.astype(jnp.bfloat16) if jnp.issubdtype(t.dtype, jnp.floating) else t)(jnp.asarray(a)))
    B, F, D, L = 4096, 26, 128, 6
    Din = min(F * D, 1024)
    return {
        "x0": _w((lambda *s: _rng.normal(s) * 0.05)(B, Din)),
        "ws": _w((lambda *s: _rng.normal(s) * 0.05)(L, Din, Din)),
        "bs": _w((lambda *s: _rng.normal(s) * 0.05)(L, Din)),
    }

def reference(x0, ws, bs):
    x = x0
    for l in range(ws.shape[0]):
        x = x0 * (x @ ws[l] + bs[l]) + x
    return x
```

```python
import jax
import jax.numpy as jnp
import jax.experimental.pallas as pl
import jax.experimental.pallas.tpu as pltpu

_F32 = jnp.float32

_R1 = 736
_SUBS = (432, 128)
_KCHUNKS = (128, 128, 256, 512)
_TAIL = (512, 256, 128, 128)
_WPAD = 128


def _compiler_params():
    base = dict(vmem_limit_bytes=100 * 1024 * 1024)
    for extra in (
        dict(disable_bounds_checks=True, disable_semaphore_checks=True),
        dict(disable_bounds_checks=True),
        dict(),
    ):
        try:
            return pltpu.CompilerParams(**base, **extra)
        except TypeError:
            continue
    return pltpu.CompilerParams(**base)


def _kernel(x0_hbm, w_hbm, b_hbm, o_hbm,
            x0_v, w_v, b_v, b32_v, o_v, xs_v, acc_v, sem_in, sem_o):
    B, D = x0_hbm.shape
    L = w_hbm.shape[0]
    dt = x0_v.dtype
    R1, R2, nk = _R1, sum(_SUBS), len(_KCHUNKS)
    n_blocks = (B - R1) // R2
    koffs = [sum(_KCHUNKS[:i]) for i in range(nk)]
    cols = pl.ds(0, D)
    head = pl.ds(0, R1)

    def k_group(c):
        ks = pl.ds(koffs[c], _KCHUNKS[c])
        sem = sem_in.at[c % 2]
        grp = [
            pltpu.make_async_copy(x0_hbm.at[head, ks], x0_v.at[head, ks], sem),
            pltpu.make_async_copy(w_hbm.at[0, ks, :], w_v.at[0, ks, cols], sem),
        ]
        if c == 1:
            grp.append(pltpu.make_async_copy(b_hbm, b_v, sem))
        return grp

    def w_copy(l):
        return pltpu.make_async_copy(
            w_hbm.at[l], w_v.at[l, :, cols], sem_in.at[(nk - 1 + l) % 2])

    def x_rest_copy():
        rest = pl.ds(R1, B - R1)
        return pltpu.make_async_copy(
            x0_hbm.at[rest], x0_v.at[rest], sem_in.at[(nk - 1 + L) % 2])

    def group(g):
        return k_group(g) if g < nk else [w_copy(g - nk + 1)]

    for g in range(2):
        for cp in group(g):
            cp.start()

    acc = None
    for c in range(nk):
        for cp in group(c):
            cp.wait()
        for cp in group(c + 2):
            cp.start()
        if c == 1:
            for l in range(L):
                b32_v[l] = b_v[l:l + 1, :].astype(_F32)
        ks = pl.ds(koffs[c], _KCHUNKS[c])
        part = jnp.dot(x0_v[head, ks], w_v[0, ks, cols], preferred_element_type=_F32)
        if c == 0:
            acc_v[...] = part
        elif c < nk - 1:
            acc_v[...] += part
        else:
            acc = acc_v[...] + part
    x0f = x0_v[head, :].astype(_F32)
    xs_v[...] = (x0f * (acc + b32_v[0]) + x0f).astype(dt)

    def s_body(l, carry):
        w_copy(l).wait()

        @pl.when(l + 2 < L)
        def _():
            w_copy(l + 2).start()

        @pl.when(l + 2 == L)
        def _():
            x_rest_copy().start()

        x = xs_v[...]
        acc = jnp.dot(x, w_v[l, :, cols], preferred_element_type=_F32)
        x0f = x0_v[head, :].astype(_F32)
        xs_v[...] = (x0f * (acc + b32_v[l]) + x.astype(_F32)).astype(dt)
        return carry

    jax.lax.fori_loop(1, L, s_body, 0)
    pltpu.make_async_copy(xs_v, o_hbm.at[head], sem_o).start()
    x_rest_copy().wait()

    def m_body(i, carry):
        off = 0
        for si, rs in enumerate(_SUBS):
            q0 = pl.multiple_of(i * R2 + off, 16)
            r0 = pl.multiple_of(R1 + i * R2 + off, 16)
            x = x0_v[pl.ds(r0, rs), :]
            x0f = x.astype(_F32)
            for l in range(L - 1):
                acc = jnp.dot(x, w_v[l, :, cols], preferred_element_type=_F32)
                x = (x0f * (acc + b32_v[l]) + x.astype(_F32)).astype(dt)
            c0 = 0
            for cw in (_TAIL if si == len(_SUBS) - 1 else (D,)):
                cs = pl.ds(c0, cw)
                acc = jnp.dot(x, w_v[L - 1, :, cs], preferred_element_type=_F32)
                y = (x0f[:, c0:c0 + cw] * (acc + b32_v[L - 1, :, cs])
                     + x[:, c0:c0 + cw].astype(_F32))
                o_v[pl.ds(q0, rs), cs] = y.astype(dt)
                pltpu.make_async_copy(
                    o_v.at[pl.ds(q0, rs), cs], o_hbm.at[pl.ds(r0, rs), cs], sem_o).start()
                c0 += cw
            off += rs
        return carry

    jax.lax.fori_loop(0, n_blocks, m_body, 0)
    pltpu.make_async_copy(x0_v, o_hbm, sem_o).wait()


@jax.jit
def pallas_standalone__dcn_v2_cross__recsys_kernel(
    x0: jax.Array,
    ws: jax.Array,
    bs: jax.Array,
):
    B, D = x0.shape
    L = ws.shape[0]
    R1, R2 = _R1, sum(_SUBS)
    assert ws.shape == (L, D, D) and bs.shape == (L, D) and L >= 3
    assert (B - R1) % R2 == 0 and sum(_KCHUNKS) == D and sum(_TAIL) == D
    assert R1 % 16 == 0 and all(s % 16 == 0 for s in _SUBS)

    return pl.pallas_call(
        _kernel,
        in_specs=[pl.BlockSpec(memory_space=pl.ANY)] * 3,
        out_specs=pl.BlockSpec(memory_space=pl.ANY),
        out_shape=jax.ShapeDtypeStruct((B, D), x0.dtype),
        scratch_shapes=[
            pltpu.VMEM((B, D), x0.dtype),
            pltpu.VMEM((L, D, D + _WPAD), ws.dtype),
            pltpu.VMEM((L, D), bs.dtype),
            pltpu.VMEM((L, 1, D), _F32),
            pltpu.VMEM((B - R1, D), x0.dtype),
            pltpu.VMEM((R1, D), x0.dtype),
            pltpu.VMEM((R1, D), _F32),
            pltpu.SemaphoreType.DMA((2,)),
            pltpu.SemaphoreType.DMA(()),
        ],
        compiler_params=_compiler_params(),
    )(x0, ws, bs)
```

```python
import jax
import jax.numpy as jnp
import jax.experimental.pallas as pl
import jax.experimental.pallas.tpu as pltpu

_F32 = jnp.float32

_R1 = 736
_R2 = 560
_NS = 2
_KCHUNKS = (128, 128, 256, 512)
_TAIL = (512, 256, 128, 128)
_LAST_ROWS = 128
_PAD = 128
_PIN = 16


def _compiler_params():
    base = dict(vmem_limit_bytes=100 * 1024 * 1024)
    for extra in (
        dict(disable_bounds_checks=True, disable_semaphore_checks=True),
        dict(disable_bounds_checks=True),
    ):
        try:
            return pltpu.CompilerParams(**base, **extra)
        except TypeError:
            continue
    return pltpu.CompilerParams(**base)


def _kernel(x0_hbm, w_hbm, b_hbm, o_hbm,
            x0_v, w_v, b_v, b32_v, o_v, xs_v, acc_v, xin_v, xt_v, we_v,
            sem_k, sem_w, sem_x, sem_o):
    B, D = x0_hbm.shape
    L = w_hbm.shape[0]
    dt = x0_v.dtype
    R1, R2, NS, nk = _R1, _R2, _NS, len(_KCHUNKS)
    RP = R1 // 2
    n_blk = (B - R1) // R2
    n_rem = L - 1 - NS
    koffs = [sum(_KCHUNKS[:i]) for i in range(nk)]
    cols = pl.ds(0, D)
    head = pl.ds(0, R1)
    h1 = pl.ds(0, RP)
    h2 = pl.ds(RP, RP)

    def k_group(c):
        ks = pl.ds(koffs[c], _KCHUNKS[c])
        grp = [
            pltpu.make_async_copy(w_hbm.at[0, ks, :], w_v.at[0, ks, cols], sem_k.at[c]),
            pltpu.make_async_copy(x0_hbm.at[head, ks], x0_v.at[:, ks], sem_k.at[c]),
        ]
        if c == 1:
            grp.append(pltpu.make_async_copy(b_hbm, b_v, sem_k.at[c]))
        return grp

    def w_copy(l):
        return pltpu.make_async_copy(w_hbm.at[l], w_v.at[l, :, cols], sem_w.at[l])

    def w_hi_copy():
        hi = pl.ds(NS + 1, n_rem)
        return pltpu.make_async_copy(w_hbm.at[hi], w_v.at[hi, :, cols], sem_w.at[0])

    def x_blk_copy(i):
        rows = pl.ds(pl.multiple_of(R1 + i * R2, 16), R2)
        return pltpu.make_async_copy(x0_hbm.at[rows], xin_v.at[pl.ds(0, R2)], sem_x.at[0])

    def head_layer(i):
        return NS + 1 + jnp.where(i >= n_rem, i - n_rem, i)

    def we_copy(i):
        return pltpu.make_async_copy(
            w_hbm.at[head_layer(i)], we_v.at[pl.ds(0, D), cols], sem_x.at[1])

    def group(g):
        return k_group(g) if g < nk else [w_copy(g - nk + 1)]

    def _bias_via(buf, row0, l):
        spare = pl.ds(row0, _PIN)
        buf[spare, cols] = jnp.broadcast_to(b_v[l:l + 1, :], (_PIN, D))
        return buf[spare, cols][0:1, :].astype(_F32)

    for g in range(2):
        for cp in group(g):
            cp.start()

    acc = None
    for c in range(nk):
        for cp in group(c):
            cp.wait()
        for cp in group(c + 2):
            cp.start()
        if c == 1:
            for l in range(L):
                b32_v[l] = b_v[l:l + 1, :].astype(_F32)
        ks = pl.ds(koffs[c], _KCHUNKS[c])
        part = jnp.dot(x0_v[:, ks], w_v[0, ks, cols], preferred_element_type=_F32)
        if c == 0:
            acc_v[...] = part
        elif c < nk - 1:
            acc_v[...] += part
        else:
            acc = acc_v[...] + part
    x0f = x0_v[...].astype(_F32)
    xs_v[...] = (x0f * (acc + b32_v[0]) + x0f).astype(dt)

    def s_body(l, carry):
        w_copy(l).wait()

        @pl.when(l == 1)
        def _():
            w_hi_copy().start()

        @pl.when(l == NS)
        def _():
            x_blk_copy(0).start()
            we_copy(0).start()

        x = xs_v[...]
        acc = jnp.dot(x, w_v[l, :, cols], preferred_element_type=_F32)
        x0f = x0_v[...].astype(_F32)
        xs_v[...] = (x0f * (acc + b32_v[l]) + x.astype(_F32)).astype(dt)
        return carry

    jax.lax.fori_loop(1, NS + 1, s_body, 0)
    w_hi_copy().wait()

    def m_body(i, carry):
        x_blk_copy(i).wait()
        we_copy(i).wait()

        second = i >= n_rem
        le = head_layer(i)
        x = jnp.where(i == n_rem, xs_v[h2, :], xs_v[h1, :])
        acc = jnp.dot(x, we_v[pl.ds(0, D), cols], preferred_element_type=_F32)

        @pl.when(i + 1 < n_blk)
        def _():
            we_copy(i + 1).start()

        x0f = jnp.where(second, x0_v[h2, :], x0_v[h1, :]).astype(_F32)
        y = (x0f * (acc + b32_v[le]) + x.astype(_F32)).astype(dt)
        xs_v[h1, :] = y
        erows = pl.ds(pl.multiple_of(jnp.where(second, RP, 0), 16), RP)
        o_v[erows, :] = y

        @pl.when(le == L - 1)
        def _():
            pltpu.make_async_copy(o_v.at[erows], o_hbm.at[erows], sem_o).start()

        r0 = pl.multiple_of(R1 + i * R2, 16)
        x = xin_v[pl.ds(0, R2), :]
        x0f = x.astype(_F32)

        @pl.when(i + 1 < n_blk)
        def _():
            x_blk_copy(i + 1).start()

        for l in range(L - 1):
            acc = jnp.dot(x, w_v[l, :, cols], preferred_element_type=_F32)
            if l == 2:
                bl = _bias_via(xin_v, R2, l)
            elif l == 1:
                bl = _bias_via(we_v, D, l)
            else:
                bl = b32_v[l]
            xt_v[l % 2, :, cols] = (x0f * (acc + bl) + x.astype(_F32)).astype(dt)
            x = xt_v[l % 2, :, cols]

        c0 = 0
        for ci, cw in enumerate(_TAIL):
            cs = pl.ds(c0, cw)
            parts = [(0, R2)]
            if ci == len(_TAIL) - 1:
                parts = [(0, R2 - _LAST_ROWS), (R2 - _LAST_ROWS, _LAST_ROWS)]
            for ra, rn in parts:
                acc = jnp.dot(x[ra:ra + rn], w_v[L - 1, :, cs], preferred_element_type=_F32)
                y = (x0f[ra:ra + rn, c0:c0 + cw] * (acc + b32_v[L - 1, :, cs])
                     + x[ra:ra + rn, c0:c0 + cw].astype(_F32)).astype(dt)
                orows = pl.ds(pl.multiple_of(r0 + ra, 16), rn)
                o_v[orows, cs] = y
                pltpu.make_async_copy(o_v.at[orows, cs], o_hbm.at[orows, cs], sem_o).start()
            c0 += cw
        return carry

    jax.lax.fori_loop(0, n_blk, m_body, 0)
    pltpu.make_async_copy(o_v, o_hbm, sem_o).wait()


@jax.jit
def pallas_standalone__dcn_v2_cross__recsys_kernel(
    x0: jax.Array,
    ws: jax.Array,
    bs: jax.Array,
):
    B, D = x0.shape
    L = ws.shape[0]
    assert ws.shape == (L, D, D) and bs.shape == (L, D)
    assert _NS == 2 and B == _R1 + 2 * (L - 1 - _NS) * _R2
    assert sum(_KCHUNKS) == D and sum(_TAIL) == D
    assert _R1 % 32 == 0 and _R2 % 16 == 0 and _LAST_ROWS % 16 == 0
    dt = x0.dtype

    return pl.pallas_call(
        _kernel,
        in_specs=[pl.BlockSpec(memory_space=pl.ANY)] * 3,
        out_specs=pl.BlockSpec(memory_space=pl.ANY),
        out_shape=jax.ShapeDtypeStruct((B, D), dt),
        scratch_shapes=[
            pltpu.VMEM((_R1, D), dt),
            pltpu.VMEM((L, D, D + _PAD), dt),
            pltpu.VMEM((L, D), dt),
            pltpu.VMEM((L, 1, D), _F32),
            pltpu.VMEM((B, D), dt),
            pltpu.VMEM((_R1, D), dt),
            pltpu.VMEM((_R1, D), _F32),
            pltpu.VMEM((_R2 + _PIN, D), dt),
            pltpu.VMEM((2, _R2, D + _PAD), dt),
            pltpu.VMEM((D + _PIN, D + _PAD), dt),
            pltpu.SemaphoreType.DMA((len(_KCHUNKS),)),
            pltpu.SemaphoreType.DMA((_NS + 1,)),
            pltpu.SemaphoreType.DMA((2,)),
            pltpu.SemaphoreType.DMA(()),
        ],
        compiler_params=_compiler_params(),
    )(x0, ws, bs)
```

```python
import jax
import jax.numpy as jnp
import jax.experimental.pallas as pl
import jax.experimental.pallas.tpu as pltpu

_F32 = jnp.float32

_R1 = 736
_R2 = 560
_NS = 2
_KCHUNKS = (128, 128, 256, 512)
_TAIL = (512, 256, 128, 128)
_LAST_ROWS = 128
_PAD = 128
_PIN = 16


def _compiler_params():
    base = dict(vmem_limit_bytes=100 * 1024 * 1024)
    for extra in (
        dict(disable_bounds_checks=True, disable_semaphore_checks=True),
        dict(disable_bounds_checks=True),
    ):
        try:
            return pltpu.CompilerParams(**base, **extra)
        except TypeError:
            continue
    return pltpu.CompilerParams(**base)


def _kernel(x0_hbm, w_hbm, b_hbm, o_hbm,
            x0_v, w_v, b_v, b32_v, o_v, xs_v, acc_v, xin_v, xt_v, we_v,
            sem_k, sem_w, sem_x, sem_o):
    B, D = x0_hbm.shape
    L = w_hbm.shape[0]
    dt = x0_v.dtype
    R1, R2, NS, nk = _R1, _R2, _NS, len(_KCHUNKS)
    RP = R1 // 2
    n_blk = (B - R1) // R2
    n_rem = L - 1 - NS
    koffs = [sum(_KCHUNKS[:i]) for i in range(nk)]
    cols = pl.ds(0, D)
    head = pl.ds(0, R1)
    h1 = pl.ds(0, RP)
    h2 = pl.ds(RP, RP)

    def k_group(c):
        ks = pl.ds(koffs[c], _KCHUNKS[c])
        grp = [
            pltpu.make_async_copy(w_hbm.at[0, ks, :], w_v.at[0, ks, cols], sem_k.at[c]),
            pltpu.make_async_copy(x0_hbm.at[head, ks], x0_v.at[:, ks], sem_k.at[c]),
        ]
        if c == 1:
            grp.append(pltpu.make_async_copy(b_hbm, b_v, sem_k.at[c]))
        return grp

    def w_copy(l):
        return pltpu.make_async_copy(w_hbm.at[l], w_v.at[l, :, cols], sem_w.at[l])

    def w_hi_copy():
        hi = pl.ds(NS + 1, n_rem)
        return pltpu.make_async_copy(w_hbm.at[hi], w_v.at[hi, :, cols], sem_w.at[0])

    def x_blk_copy(i):
        start = R1 + i * R2
        rows = pl.ds(start if isinstance(i, int) else pl.multiple_of(start, 16), R2)
        return pltpu.make_async_copy(x0_hbm.at[rows], xin_v.at[pl.ds(0, R2)], sem_x)

    def head_layer(i):
        if isinstance(i, int):
            return NS + 1 + i % n_rem
        return NS + 1 + jnp.where(i >= n_rem, i - n_rem, i)

    def we_copy(i):
        return pltpu.make_async_copy(
            w_hbm.at[head_layer(i)], we_v.at[pl.ds(0, D), cols], sem_x)

    def group(g):
        if g < nk:
            return k_group(g)
        return [w_copy(g - nk + 1)] if g - nk + 1 <= NS else [w_hi_copy()]

    def _bias_via(buf, row0, l):
        spare = pl.ds(row0, _PIN)
        buf[spare, cols] = jnp.broadcast_to(b_v[l:l + 1, :], (_PIN, D))
        return buf[spare, cols][0:1, :].astype(_F32)

    for g in range(3):
        for cp in group(g):
            cp.start()

    acc = None
    for c in range(nk):
        for cp in group(c):
            cp.wait()
        if c == 1:
            for l in range(L):
                b32_v[l] = b_v[l:l + 1, :].astype(_F32)
        ks = pl.ds(koffs[c], _KCHUNKS[c])
        part = jnp.dot(x0_v[:, ks], w_v[0, ks, cols], preferred_element_type=_F32)
        if c == 0:
            acc_v[...] = part
        elif c < nk - 1:
            acc_v[...] += part
        else:
            acc = acc_v[...] + part
            x0f = x0_v[...].astype(_F32)
            xs_v[...] = (x0f * (acc + b32_v[0]) + x0f).astype(dt)
        for cp in group(c + 3):
            cp.start()

    def s_body(l, carry):
        w_copy(l).wait()

        @pl.when(l == 1)
        def _():
            x_blk_copy(0).start()
            we_copy(0).start()

        x = xs_v[...]
        acc = jnp.dot(x, w_v[l, :, cols], preferred_element_type=_F32)
        x0f = x0_v[...].astype(_F32)
        xs_v[...] = (x0f * (acc + b32_v[l]) + x.astype(_F32)).astype(dt)
        return carry

    jax.lax.fori_loop(1, NS + 1, s_body, 0)
    w_hi_copy().wait()

    def m_body(i, carry):
        x_blk_copy(0).wait()
        we_copy(0).wait()

        second = i >= n_rem
        le = head_layer(i)
        x = jnp.where(i == n_rem, xs_v[h2, :], xs_v[h1, :])
        acc = jnp.dot(x, we_v[pl.ds(0, D), cols], preferred_element_type=_F32)

        @pl.when(i + 1 < n_blk)
        def _():
            we_copy(i + 1).start()

        x0f = jnp.where(second, x0_v[h2, :], x0_v[h1, :]).astype(_F32)
        y = (x0f * (acc + b32_v[le]) + x.astype(_F32)).astype(dt)
        xs_v[h1, :] = y
        erows = pl.ds(pl.multiple_of(jnp.where(second, RP, 0), 16), RP)
        o_v[erows, :] = y

        @pl.when(le == L - 1)
        def _():
            pltpu.make_async_copy(o_v.at[erows], o_hbm.at[erows], sem_o).start()

        r0 = pl.multiple_of(R1 + i * R2, 16)
        x = xin_v[pl.ds(0, R2), :]
        x0f = x.astype(_F32)

        @pl.when(i + 1 < n_blk)
        def _():
            x_blk_copy(i + 1).start()

        for l in range(L - 1):
            acc = jnp.dot(x, w_v[l, :, cols], preferred_element_type=_F32)
            if l == 2:
                bl = _bias_via(xin_v, R2, l)
            elif l == 1:
                bl = _bias_via(we_v, D, l)
            else:
                bl = b32_v[l]
            xt_v[l % 2, :, cols] = (x0f * (acc + bl) + x.astype(_F32)).astype(dt)
            x = xt_v[l % 2, :, cols]

        c0 = 0
        for ci, cw in enumerate(_TAIL):
            cs = pl.ds(c0, cw)
            parts = [(0, R2)]
            if ci == len(_TAIL) - 1:
                parts = [(0, R2 - _LAST_ROWS), (R2 - _LAST_ROWS, _LAST_ROWS)]
            for ra, rn in parts:
                acc = jnp.dot(x[ra:ra + rn], w_v[L - 1, :, cs], preferred_element_type=_F32)
                y = (x0f[ra:ra + rn, c0:c0 + cw] * (acc + b32_v[L - 1, :, cs])
                     + x[ra:ra + rn, c0:c0 + cw].astype(_F32)).astype(dt)
                orows = pl.ds(pl.multiple_of(r0 + ra, 16), rn)
                o_v[orows, cs] = y
                pltpu.make_async_copy(o_v.at[orows, cs], o_hbm.at[orows, cs], sem_o).start()
            c0 += cw
        return carry

    jax.lax.fori_loop(0, n_blk, m_body, 0)
    pltpu.make_async_copy(o_v, o_hbm, sem_o).wait()


@jax.jit
def pallas_standalone__dcn_v2_cross__recsys_kernel(
    x0: jax.Array,
    ws: jax.Array,
    bs: jax.Array,
):
    B, D = x0.shape
    L = ws.shape[0]
    assert ws.shape == (L, D, D) and bs.shape == (L, D)
    assert _NS == 2 and B == _R1 + 2 * (L - 1 - _NS) * _R2
    assert sum(_KCHUNKS) == D and sum(_TAIL) == D
    assert _R1 % 32 == 0 and _R2 % 16 == 0 and _LAST_ROWS % 16 == 0
    dt = x0.dtype

    return pl.pallas_call(
        _kernel,
        in_specs=[pl.BlockSpec(memory_space=pl.ANY)] * 3,
        out_specs=pl.BlockSpec(memory_space=pl.ANY),
        out_shape=jax.ShapeDtypeStruct((B, D), dt),
        scratch_shapes=[
            pltpu.VMEM((_R1, D), dt),
            pltpu.VMEM((L, D, D + _PAD), dt),
            pltpu.VMEM((L, D), dt),
            pltpu.VMEM((L, 1, D), _F32),
            pltpu.VMEM((B, D), dt),
            pltpu.VMEM((_R1, D), dt),
            pltpu.VMEM((_R1, D), _F32),
            pltpu.VMEM((_R2 + _PIN, D), dt),
            pltpu.VMEM((2, _R2, D + _PAD), dt),
            pltpu.VMEM((D + _PIN, D + _PAD), dt),
            pltpu.SemaphoreType.DMA((len(_KCHUNKS),)),
            pltpu.SemaphoreType.DMA((_NS + 1,)),
            pltpu.SemaphoreType.DMA(()),
            pltpu.SemaphoreType.DMA(()),
        ],
        compiler_params=_compiler_params(),
    )(x0, ws, bs)
```
